```python
import os as _os
_os.environ.setdefault("JAX_PLATFORMS", "cpu")
import jax
import jax.numpy as jnp

def _softmax(x, axis=-1):
    return jax.nn.softmax(x, axis=axis)
def _gelu(x):
    return jax.nn.gelu(x, approximate=True)
def _silu(x):
    return jax.nn.silu(x)
def _sigmoid(x):
    return jax.nn.sigmoid(x)
def _layernorm(x, axis=-1, eps=1e-5):
    m = jnp.mean(x, axis=axis, keepdims=True)
    v = jnp.var(x, axis=axis, keepdims=True)
    return (x - m) / jnp.sqrt(v + eps)
def _scatter_add(tgt, idx, src, axis=0):
    return tgt.at[idx].add(src)
def _segment_sum(src, seg, n):
    return jax.ops.segment_sum(src, seg, n)
class _Rng:
    def __init__(self, key):
        self._k = key
    def _next(self):
        self._k, sub = jax.random.split(self._k)
        return sub
    def normal(self, shape):
        return jax.random.normal(self._next(), shape, dtype=jnp.bfloat16)
    def randint(self, lo, hi, shape):
        return jax.random.randint(self._next(), shape, lo, hi, dtype=jnp.int32)
    def uniform(self, shape, lo=0.0, hi=1.0):
        return jax.random.uniform(self._next(), shape, jnp.bfloat16, lo, hi)
    def permutation(self, n):
        return jax.random.permutation(self._next(), n)


kernel_name = 'parallel_sum__softmax_full_mha__moe_arch_mod__prompt'

def setup_inputs():
    _rng = _Rng(jax.random.key(int.from_bytes(__import__("os").urandom(4), "little")))
    _w = (lambda a: (lambda t: t.astype(jnp.bfloat16) if jnp.issubdtype(t.dtype, jnp.floating) else t)(jnp.asarray(a)))
    def _A_setup():
        B, S, D = 1, 2048, 512
        return {
            "x": _w((lambda *s: _rng.normal(s) * 0.05)(B, S, D)),
            "wqkv": _w((lambda *s: _rng.normal(s) * 0.1)(D, 3 * D)),
            "wo": _w((lambda *s: _rng.normal(s) * 0.05)(D, D)),
        }
    _A_in = _A_setup()

    def _B_setup():
        B, S, D, F, C = 1, 2048, 512, 1792, 1
        return {
            "x": _w((lambda *s: _rng.normal(s) * 0.05)(B, S, D)),
            "w_r": _w((lambda *s: _rng.normal(s) * 1.6)(D)),
            "w_gate": _w((lambda *s: _rng.normal(s) * 0.1)(D, F)),
            "w_up": _w((lambda *s: _rng.normal(s) * 0.1)(D, F)),
            "w_down": _w((lambda *s: _rng.normal(s) * 0.1)(F, D)),
        }
    _B_in = _B_setup()

    return {
        "A_x": _A_in["x"],
        "A_wqkv": _A_in["wqkv"],
        "A_wo": _A_in["wo"],
        "B_x": _B_in["x"],
        "B_w_r": _B_in["w_r"],
        "B_w_gate": _B_in["w_gate"],
        "B_w_up": _B_in["w_up"],
        "B_w_down": _B_in["w_down"],
    }

def reference(A_x, A_wqkv, A_wo, B_x, B_w_r, B_w_gate, B_w_up, B_w_down):
    def _A_ref(x, wqkv, wo):
        B, S, D = x.shape
        H = 32; Dh = D // H
        qkv = (lambda x, *d: x.transpose(*d))((x @ wqkv).reshape(B, S, 3, H, Dh), 2, 0, 3, 1, 4)
        q, k, v = qkv[0], qkv[1], qkv[2]
        scale = Dh ** -0.5
        scores = jnp.einsum("bhqd,bhkd->bhqk", q, k) * scale
        p = _softmax(scores, axis=-1)
        o = jnp.einsum("bhqk,bhkd->bhqd", p, v)
        return (lambda x, *d: x.transpose(*d))(o, 0, 2, 1, 3).reshape(B, S, D) @ wo

    def _B_ref(x, w_r, w_gate, w_up, w_down):
        B, S, D = x.shape
        C = 1
        r = x @ w_r
        idx = jnp.argsort(-r, axis=-1)[:, :C]
        idx_e = jnp.repeat(idx.reshape(B, C, 1), D, axis=2)
        x_sel = jnp.take_along_axis(x, idx_e, axis=1)
        g = _silu(x_sel @ w_gate)
        u = x_sel @ w_up
        y = (g * u) @ w_down
        r_sel = _sigmoid(jnp.take_along_axis(r, idx, axis=1))
        y = y * r_sel.reshape(B, C, 1)
        b_off = (jnp.arange(B) * S).reshape(B, 1)
        flat_idx = (idx + b_off).reshape(B * C)
        zero = (x * 0.0).reshape(B * S, D)
        upd = _scatter_add(zero, flat_idx, y.reshape(B * C, D), axis=0)
        return x + upd.reshape(B, S, D)

    x = A_x
    xn = _layernorm(x, axis=-1)
    return x + _A_ref(xn, A_wqkv, A_wo) + _B_ref(xn, B_w_r, B_w_gate, B_w_up, B_w_down)
```

```python
import functools
import math

import jax
import jax.numpy as jnp
from jax import lax
import jax.experimental.pallas as pl
import jax.experimental.pallas.tpu as pltpu

_F32 = jnp.float32
_BF16 = jnp.bfloat16

_NT = (((1,), (1,)), ((), ()))


def _rb(v):
    return v.astype(_BF16).astype(_F32)


def _same(m, dep):
    return jnp.maximum(m, jnp.minimum(dep, m))


def _kernel(x_ref, wqkv_ref, wo_ref, wr_ref, wg_hbm, wu_hbm, wd_hbm, o_ref,
            xn_scr, qt_scr, k_scr, vt_scr, wqvt_scr, wot_scr, at_scr,
            s0, s1, m0, m1, l_scr, oa_scr, y_scr, idx_scr,
            wg_v, wu_v, wd_v, sems, *, S, D, H, TQ, TC, KC, SKEW, DEP, DEPO):
    Dh = D // H
    HG = 128 // Dh
    NG = D // 128
    NQ = S // TQ
    NC = S // KC
    step = pl.program_id(0)
    qscale = float(Dh) ** -0.5 * math.log2(math.e)
    sb, mb = (s0, s1), (m0, m1)

    def ffn_copies():
        return (pltpu.make_async_copy(wg_hbm, wg_v, sems.at[0]),
                pltpu.make_async_copy(wu_hbm, wu_v, sems.at[1]),
                pltpu.make_async_copy(wd_hbm, wd_v, sems.at[2]))

    @pl.when(step == 0)
    def _prologue():
        for c in ffn_copies():
            c.start()

        s0[...] = jnp.zeros_like(s0)
        s1[...] = jnp.zeros_like(s1)
        m0[...] = jnp.zeros_like(m0)
        m1[...] = jnp.zeros_like(m1)
        l_scr[...] = jnp.ones_like(l_scr)
        oa_scr[...] = jnp.zeros_like(oa_scr)

        wqvt_scr[0:D, :] = wqkv_ref[:, 0:D].astype(_F32).T.astype(_BF16)
        wqvt_scr[D:2 * D, :] = wqkv_ref[:, 2 * D:3 * D].astype(_F32).T.astype(_BF16)
        wot_scr[...] = wo_ref[...].astype(_F32).T.astype(_BF16)

        def layernorm(c):
            rows = pl.ds(c * TC, TC)
            xf = x_ref[rows, :].astype(_F32)
            mu = jnp.mean(xf, axis=-1, keepdims=True)
            xc = xf - mu
            var = jnp.mean(xc * xc, axis=-1, keepdims=True)
            den = _rb(jnp.sqrt(_rb(_rb(var) + 1e-5)))
            xn = _rb(xf - _rb(mu)) / den
            xn_scr[rows, :] = xn.astype(_BF16)

        def project(c):
            rows = pl.ds(c * TC, TC)
            xn = xn_scr[rows, :]
            k = jnp.dot(xn, wqkv_ref[:, D:2 * D], preferred_element_type=_F32)
            k_scr[rows, :] = k.astype(_BF16)
            qt = lax.dot_general(wqvt_scr[0:D, :], xn, _NT,
                                 preferred_element_type=_F32)
            qt_scr[:, rows] = (_rb(qt) * qscale).astype(_BF16)
            vt = lax.dot_general(wqvt_scr[D:2 * D, :], xn, _NT,
                                 preferred_element_type=_F32)
            vt_scr[:, rows] = vt.astype(_BF16)

        layernorm(0)
        for c in range(S // TC):
            if c + 1 < S // TC:
                layernorm(c + 1)
            project(c)

        xn_all = xn_scr[...]
        wr = jnp.broadcast_to(wr_ref[...], (16, D))
        r = _rb(lax.dot_general(wr, xn_all, _NT, preferred_element_type=_F32))
        rmax = jnp.max(r, axis=-1, keepdims=True)
        col = lax.broadcasted_iota(jnp.int32, (16, S), 1)
        idx = jnp.min(jnp.where(r == rmax, col, S), axis=-1, keepdims=True)
        idx_scr[...] = jnp.broadcast_to(idx[0:8, :], (8, 128))
        onehot = jnp.where(col == idx, 1.0, 0.0).astype(_BF16)
        xsel = jnp.dot(onehot, xn_all, preferred_element_type=_F32).astype(_BF16)

        for c in ffn_copies():
            c.wait()
        g = _rb(jnp.dot(xsel, wg_v[...], preferred_element_type=_F32))
        g = _rb(g * _rb(jax.nn.sigmoid(g)))
        u = _rb(jnp.dot(xsel, wu_v[...], preferred_element_type=_F32))
        gu = (g * u).astype(_BF16)
        y = _rb(jnp.dot(gu, wd_v[...], preferred_element_type=_F32))
        y = _rb(y * _rb(jax.nn.sigmoid(rmax)))
        y_scr[...] = y[0:8, :]

    q0 = pl.multiple_of(jnp.minimum(step, NQ - 1) * TQ, TQ)

    def run(g, do_a, nslots):
        h_base = g * HG
        gbase = step * H + h_base
        lacc, oacc = l_scr[...], oa_scr[...]
        w = macc = mB = None
        hist, histo = [], []
        c0 = pl.multiple_of(g * 128, 128)
        for n in range(nslots):
            j, c = divmod(n, NC)
            if do_a:
                if c == 0:
                    r0a = pl.multiple_of((h_base + j) * Dh, Dh)
                    qrow = qt_scr[pl.ds(r0a, Dh), pl.ds(q0, TQ)]
                    parts = []
                    if j > 0:
                        parts.append(jnp.zeros((j * Dh, TQ), _BF16))
                    parts.append(qrow)
                    if j < HG - 1:
                        parts.append(jnp.zeros(((HG - 1 - j) * Dh, TQ), _BF16))
                    w = jnp.concatenate(parts, axis=0)
                    macc = None
                rows = pl.ds(c * KC, KC)
                s = jnp.dot(k_scr[rows, pl.ds(c0, 128)], w,
                            preferred_element_type=_F32)
                sb[j % 2][rows, :] = s
                for r in range(KC // 8):
                    sr = s[r * 8:(r + 1) * 8, :]
                    macc = sr if macc is None else jnp.maximum(macc, sr)
                if c == NC - 1:
                    mb[j % 2][...] = jnp.broadcast_to(
                        jnp.max(macc, axis=0, keepdims=True), (8, TQ))
            jb, cb = divmod(n - NC - SKEW, NC)
            gB = gbase + jb + 2 * H
            r0 = pl.multiple_of((gB % H) * Dh, Dh)
            if cb == 0 or mB is None:
                mB = mb[jb % 2][...]
            if cb == 0:
                lacc = None
                oacc = None
            mcur = mB
            if len(hist) >= DEP:
                mcur = _same(mcur, hist[-DEP])
            if len(histo) >= DEPO:
                mcur = _same(mcur, histo[-DEPO])
            rows = pl.ds(cb * KC, KC)
            p = jnp.exp2(sb[jb % 2][rows, :].reshape(KC // 8, 8, TQ)
                         - mcur[None]).reshape(KC, TQ)
            for r in reversed(range(KC // 8)):
                pr = p[r * 8:(r + 1) * 8, :]
                lacc = pr if lacc is None else lacc + pr
            hist.append(lacc)
            oc = jnp.dot(vt_scr[pl.ds(r0, Dh), rows], p.astype(_BF16),
                         preferred_element_type=_F32)
            oacc = oc if oacc is None else oacc + oc
            histo.append(oc[0:8, :])
            if cb == NC - 1:
                l = jnp.sum(lacc, axis=0, keepdims=True)
                par = (gB // H) % 2
                at_scr[par, pl.ds(r0, Dh), :] = (oacc / l).astype(_BF16)
        l_scr[...] = lacc
        oa_scr[...] = oacc

    def finish_block():
        qp = pl.multiple_of((step - 1) * TQ, TQ)
        par = (step - 1) % 2
        outt = jnp.dot(wot_scr[...], at_scr[par], preferred_element_type=_F32)
        a = _rb(outt.T)
        xb = x_ref[pl.ds(qp, TQ), :].astype(_F32)
        xnb = xn_scr[pl.ds(qp, TQ), :].astype(_F32)
        rows = lax.broadcasted_iota(jnp.int32, (TQ, D), 0) + qp
        upd = jnp.where(rows == idx_scr[0:1, 0:1], y_scr[0:1, :], 0.0)
        o_ref[...] = (_rb(xb + a) + _rb(xnb + upd)).astype(o_ref.dtype)

    @pl.when(step < NQ)
    def _main():
        def body(g, carry):
            run(g, True, HG * NC)

            @pl.when(jnp.logical_and(g == 0, step > 0))
            def _():
                finish_block()
            return carry
        lax.fori_loop(0, NG, body, 0)

    @pl.when(step == NQ)
    def _tail():
        run(0, False, NC + SKEW)
        finish_block()


@jax.jit
def pallas_parallel_sum__softmax_full_mha__moe_arch_mod__prompt_kernel(
    A_x: jax.Array,
    A_wqkv: jax.Array,
    A_wo: jax.Array,
    B_x: jax.Array,
    B_w_r: jax.Array,
    B_w_gate: jax.Array,
    B_w_up: jax.Array,
    B_w_down: jax.Array,
):
    del B_x
    B, S, D = A_x.shape
    assert B == 1
    F = B_w_gate.shape[1]
    H = 32
    TQ = 512
    NQ = S // TQ
    Dh = D // H

    x2 = A_x.reshape(S, D)
    wr2 = B_w_r.reshape(1, D)

    full = lambda shape: pl.BlockSpec(shape, lambda i: (0,) * len(shape))
    kern = functools.partial(_kernel, S=S, D=D, H=H, TQ=TQ, TC=256, KC=128,
                             SKEW=2, DEP=2, DEPO=3)
    out = pl.pallas_call(
        kern,
        grid=(NQ + 1,),
        in_specs=[
            full((S, D)),
            full((D, 3 * D)),
            full((D, D)),
            full((1, D)),
            pl.BlockSpec(memory_space=pl.ANY),
            pl.BlockSpec(memory_space=pl.ANY),
            pl.BlockSpec(memory_space=pl.ANY),
        ],
        out_specs=pl.BlockSpec((TQ, D), lambda i: (jnp.maximum(i - 1, 0), 0)),
        out_shape=jax.ShapeDtypeStruct((S, D), A_x.dtype),
        scratch_shapes=[
            pltpu.VMEM((S, D), _BF16),
            pltpu.VMEM((D, S), _BF16),
            pltpu.VMEM((S, D), _BF16),
            pltpu.VMEM((D, S), _BF16),
            pltpu.VMEM((2 * D, D), _BF16),
            pltpu.VMEM((D, D), _BF16),
            pltpu.VMEM((2, D, TQ), _BF16),
            pltpu.VMEM((S, TQ), _F32),
            pltpu.VMEM((S, TQ), _F32),
            pltpu.VMEM((8, TQ), _F32),
            pltpu.VMEM((8, TQ), _F32),
            pltpu.VMEM((8, TQ), _F32),
            pltpu.VMEM((Dh, TQ), _F32),
            pltpu.VMEM((8, D), _F32),
            pltpu.VMEM((8, 128), jnp.int32),
            pltpu.VMEM((D, F), _BF16),
            pltpu.VMEM((D, F), _BF16),
            pltpu.VMEM((F, D), _BF16),
            pltpu.SemaphoreType.DMA((3,)),
        ],
        compiler_params=pltpu.CompilerParams(
            dimension_semantics=("arbitrary",),
            vmem_limit_bytes=100 * 1024 * 1024,
        ),
    )(x2, A_wqkv, A_wo, wr2, B_w_gate, B_w_up, B_w_down)
    return out.reshape(B, S, D)
```

```python
import functools
import math

import jax
import jax.numpy as jnp
from jax import lax
import jax.experimental.pallas as pl
import jax.experimental.pallas.tpu as pltpu

_F32 = jnp.float32
_BF16 = jnp.bfloat16

_NT = (((1,), (1,)), ((), ()))


def _rb(v):
    return v.astype(_BF16).astype(_F32)


def _same(m, dep):
    return jnp.maximum(m, jnp.minimum(dep, m))


def _kernel(x_hbm, wqkv_hbm, wo_hbm, wr_ref, wg_hbm, wu_hbm, wd_hbm, o_hbm,
            x_scr, w3_v, wo_v, xn_scr, qt_scr, k_scr, vt_scr, wqvt_scr,
            wot_scr, at_scr, s0, s1, m0, m1, l_scr, oa_scr, r_scr, res_scr,
            o_scr, wg_v, wu_v, wd_v, sems,
            *, S, D, H, TQ, TC, KC, SKEW, DEP, DEPO, GU):
    Dh = D // H
    HG = 128 // Dh
    NG = D // 128
    NQ = S // TQ
    NC = S // KC
    NT = S // TC
    qscale = float(Dh) ** -0.5 * math.log2(math.e)
    sb, mb = (s0, s1), (m0, m1)

    def x_copy(c):
        rows = pl.ds(c * TC, TC)
        return pltpu.make_async_copy(x_hbm.at[rows, :], x_scr.at[rows, :],
                                     sems.at[c])

    def w3_copy(i):
        return pltpu.make_async_copy(wqkv_hbm.at[:, pl.ds(i * D, D)],
                                     w3_v.at[i], sems.at[NT + i])

    wo_copy = pltpu.make_async_copy(wo_hbm, wo_v, sems.at[NT + 3])
    ffn_copies = (pltpu.make_async_copy(wg_hbm, wg_v, sems.at[NT + 4]),
                  pltpu.make_async_copy(wu_hbm, wu_v, sems.at[NT + 5]),
                  pltpu.make_async_copy(wd_hbm, wd_v, sems.at[NT + 6]))

    def out_copy(i):
        rows = pl.ds(pl.multiple_of(i * 128, 128), 128)
        return pltpu.make_async_copy(o_scr.at[rows, :], o_hbm.at[rows, :],
                                     sems.at[NT + 7 + i])

    x_copy(0).start()
    w3_copy(1).start()
    x_copy(1).start()
    w3_copy(0).start()
    w3_copy(2).start()

    wr = jnp.broadcast_to(wr_ref[...].reshape(1, D), (16, D))

    def layernorm(c):
        rows = pl.ds(c * TC, TC)
        xf = x_scr[rows, :].astype(_F32)
        mu = jnp.mean(xf, axis=-1, keepdims=True)
        xc = xf - mu
        var = jnp.mean(xc * xc, axis=-1, keepdims=True)
        den = _rb(jnp.sqrt(_rb(_rb(var) + 1e-5)))
        xn = (_rb(xf - _rb(mu)) * (1.0 / den)).astype(_BF16)
        xn_scr[rows, :] = xn
        res_scr[rows, :] = xf + xn.astype(_F32)

    def router(c):
        rows = pl.ds(c * TC, TC)
        r_scr[:, rows] = _rb(lax.dot_general(wr, xn_scr[rows, :], _NT,
                                             preferred_element_type=_F32))

    def project_k(c, n=TC):
        rows = pl.ds(c * n, n)
        k = jnp.dot(xn_scr[rows, :], w3_v[1], preferred_element_type=_F32)
        k_scr[rows, :] = k.astype(_BF16)

    def project_q(c, n=TC):
        rows = pl.ds(c * n, n)
        qt = lax.dot_general(wqvt_scr[0:D, :], xn_scr[rows, :], _NT,
                             preferred_element_type=_F32)
        qt_scr[:, rows] = (qt * qscale).astype(_BF16)

    def project_v(c, n=TC):
        rows = pl.ds(c * n, n)
        vt = lax.dot_general(wqvt_scr[D:2 * D, :], xn_scr[rows, :], _NT,
                             preferred_element_type=_F32)
        vt_scr[:, rows] = vt.astype(_BF16)
        s1[rows, :] = jnp.zeros((n, TQ), _F32)

    x_copy(0).wait()
    for c in range(2, NT):
        x_copy(c).start()
    wo_copy.start()
    layernorm(0)
    w3_copy(1).wait()
    x_copy(1).wait()
    project_k(0)
    layernorm(1)
    project_k(1)
    w3_copy(0).wait()
    w3_copy(2).wait()
    wqvt_scr[0:D, :] = w3_v[0].astype(_F32).T.astype(_BF16)
    wqvt_scr[D:2 * D, :] = w3_v[2].astype(_F32).T.astype(_BF16)
    router(0)
    router(1)
    project_q(0)
    project_v(0)
    project_q(1)
    for c in range(2, NT):
        x_copy(c).wait()
    wo_copy.wait()
    for cp in ffn_copies:
        cp.start()
    wot_scr[...] = wo_v[...].astype(_F32).T.astype(_BF16)
    project_v(1)
    for c in range(2, NT):
        layernorm(c)
    for c in range(2, NT - 2):
        router(c)
        project_k(c)
        if c + 2 >= NT - 2:
            router(c + 2)
        project_q(c)
        project_v(c)
    for cp in ffn_copies:
        cp.wait()

    F = wg_v.shape[1]
    SUB = 128
    fill = []
    for c in range((NT - 2) * TC // SUB, NT * TC // SUB):
        fill += [functools.partial(f, c, SUB)
                 for f in (project_k, project_q, project_v)]

    def filler():
        if fill:
            fill.pop(0)()

    filler()
    r = r_scr[...]
    rmax = jnp.max(r, axis=-1, keepdims=True)
    col = lax.broadcasted_iota(jnp.int32, (16, S), 1)
    idx = jnp.min(jnp.where(r == rmax, col, S), axis=-1, keepdims=True)
    onehot = jnp.where(col == idx, 1.0, 0.0).astype(_BF16)
    xsel = None
    for i in range(2):
        cols = slice(i * S // 2, (i + 1) * S // 2)
        part = jnp.dot(onehot[:, cols], xn_scr[cols, :],
                       preferred_element_type=_F32)
        xsel = part if xsel is None else xsel + part
        filler()
    xsel = xsel.astype(_BF16)
    gus = []
    for i in range(2):
        cols = slice(i * F // 2, (i + 1) * F // 2)
        g = _rb(jnp.dot(xsel, wg_v[:, cols], preferred_element_type=_F32))
        g = _rb(g * _rb(jax.nn.sigmoid(g)))
        filler()
        u = _rb(jnp.dot(xsel, wu_v[:, cols], preferred_element_type=_F32))
        gus.append((g * u).astype(_BF16))
        filler()
    y = None
    for i in range(2):
        cols = slice(i * F // 2, (i + 1) * F // 2)
        part = jnp.dot(gus[i], wd_v[cols, :], preferred_element_type=_F32)
        y = part if y is None else y + part
        filler()
    y = _rb(_rb(y) * _rb(jax.nn.sigmoid(rmax)))
    idx_s = jnp.clip(jnp.min(idx), 0, S - 1)
    row = pl.ds(idx_s, 1)
    res_scr[row, :] = res_scr[row, :] + y[0:1, :]
    while fill:
        filler()
    s0[pl.ds(S - SKEW * KC, SKEW * KC), :] = jnp.zeros((SKEW * KC, TQ), _F32)
    m0[...] = jnp.zeros_like(m0)
    m1[...] = jnp.zeros_like(m1)
    l_scr[...] = jnp.ones_like(l_scr)
    oa_scr[...] = jnp.zeros_like(oa_scr)

    def run(qb, g, do_a, nslots, extra=()):
        extra = list(extra)
        h_base = g * HG
        gbase = qb * H + h_base
        lacc, oacc = l_scr[...], oa_scr[...]
        w = macc = mB = None
        hist, histo = [], []
        if do_a:
            q0 = pl.multiple_of(qb * TQ, TQ)
        for n in range(nslots):
            j, c = divmod(n, NC)
            if do_a:
                if c == 0:
                    jj = j % HG
                    c0 = pl.multiple_of((g + j // HG) * 128, 128)
                    r0a = pl.multiple_of((h_base + j) * Dh, Dh)
                    qrow = qt_scr[pl.ds(r0a, Dh), pl.ds(q0, TQ)]
                    parts = []
                    if jj > 0:
                        parts.append(jnp.zeros((jj * Dh, TQ), _BF16))
                    parts.append(qrow)
                    if jj < HG - 1:
                        parts.append(jnp.zeros(((HG - 1 - jj) * Dh, TQ), _BF16))
                    w = jnp.concatenate(parts, axis=0)
                    macc = None
                rows = pl.ds(c * KC, KC)
                s = jnp.dot(k_scr[rows, pl.ds(c0, 128)], w,
                            preferred_element_type=_F32)
                sb[j % 2][rows, :] = s
                for r in range(KC // 8):
                    sr = s[r * 8:(r + 1) * 8, :]
                    macc = sr if macc is None else jnp.maximum(macc, sr)
                if c == NC - 1:
                    mb[j % 2][...] = jnp.broadcast_to(
                        jnp.max(macc, axis=0, keepdims=True), (8, TQ))
            jb, cb = divmod(n - NC - SKEW, NC)
            gB = gbase + jb + 2 * H
            r0 = pl.multiple_of((gB % H) * Dh, Dh)
            if cb == 0 or mB is None:
                mB = mb[jb % 2][...]
            if cb == 0:
                lacc = None
                oacc = None
            mcur = mB
            if len(hist) >= DEP:
                mcur = _same(mcur, hist[-DEP])
            if len(histo) >= DEPO:
                mcur = _same(mcur, histo[-DEPO])
            rows = pl.ds(cb * KC, KC)
            p = jnp.exp2(sb[jb % 2][rows, :].reshape(KC // 8, 8, TQ)
                         - mcur[None]).reshape(KC, TQ)
            for r in reversed(range(KC // 8)):
                pr = p[r * 8:(r + 1) * 8, :]
                lacc = pr if lacc is None else lacc + pr
            hist.append(lacc)
            oc = jnp.dot(vt_scr[pl.ds(r0, Dh), rows], p.astype(_BF16),
                         preferred_element_type=_F32)
            oacc = oc if oacc is None else oacc + oc
            histo.append(oc[0:8, :])
            if cb == NC - 1:
                l = jnp.sum(lacc, axis=0, keepdims=True)
                par = (gB // H) % 2
                at_scr[par, pl.ds(r0, Dh), :] = (oacc / l).astype(_BF16)
            if extra and n % 4 == 3:
                extra.pop(0)()
        assert not extra
        l_scr[...] = lacc
        oa_scr[...] = oacc

    def finish_block(qb, k0=0):
        par = qb % 2
        for t in range(TQ // 128):
            rows = pl.ds(pl.multiple_of(qb * TQ + t * 128, 128), 128)
            outt = jnp.dot(wot_scr[:, k0:D],
                           at_scr[par, k0:D, t * 128:(t + 1) * 128],
                           preferred_element_type=_F32)
            o_scr[rows, :] = (res_scr[rows, :] + outt.T).astype(o_scr.dtype)
            out_copy(qb * (TQ // 128) + t).start()

    def early_proj(qb, k1, t):
        rows = pl.ds(qb * TQ + t * 128, 128)
        outt = jnp.dot(wot_scr[:, 0:k1],
                       at_scr[qb % 2, 0:k1, t * 128:(t + 1) * 128],
                       preferred_element_type=_F32)
        res_scr[rows, :] = res_scr[rows, :] + outt.T

    def body(t, carry):
        qb = t // (NG // GU)
        g = (t % (NG // GU)) * GU
        run(qb, g, True, GU * HG * NC)

        @pl.when(jnp.logical_and(g == 0, qb > 0))
        def _():
            finish_block(qb - 1)
        return carry

    lax.fori_loop(0, NQ * NG // GU, body, 0)
    k1 = D - 128
    run(NQ, 0, False, NC + SKEW,
        [functools.partial(early_proj, NQ - 1, k1, t) for t in range(TQ // 128)])
    finish_block(NQ - 1, k1)
    for i in range(S // 128):
        out_copy(i).wait()


@jax.jit
def pallas_parallel_sum__softmax_full_mha__moe_arch_mod__prompt_kernel(
    A_x: jax.Array,
    A_wqkv: jax.Array,
    A_wo: jax.Array,
    B_x: jax.Array,
    B_w_r: jax.Array,
    B_w_gate: jax.Array,
    B_w_up: jax.Array,
    B_w_down: jax.Array,
):
    del B_x
    B, S, D = A_x.shape
    assert B == 1
    F = B_w_gate.shape[1]
    H = 32
    TQ = 512
    TC = 256
    NQ = S // TQ
    Dh = D // H

    x2 = A_x.reshape(S, D)

    hbm = pl.BlockSpec(memory_space=pl.ANY)
    kern = functools.partial(_kernel, S=S, D=D, H=H, TQ=TQ, TC=TC, KC=128,
                             SKEW=2, DEP=2, DEPO=3, GU=1)
    out = pl.pallas_call(
        kern,
        in_specs=[hbm, hbm, hbm, pl.BlockSpec(memory_space=pltpu.VMEM),
                  hbm, hbm, hbm],
        out_specs=hbm,
        out_shape=jax.ShapeDtypeStruct((S, D), A_x.dtype),
        scratch_shapes=[
            pltpu.VMEM((S, D), _BF16),
            pltpu.VMEM((3, D, D), _BF16),
            pltpu.VMEM((D, D), _BF16),
            pltpu.VMEM((S, D), _BF16),
            pltpu.VMEM((D, S), _BF16),
            pltpu.VMEM((S, D), _BF16),
            pltpu.VMEM((D, S), _BF16),
            pltpu.VMEM((2 * D, D), _BF16),
            pltpu.VMEM((D, D), _BF16),
            pltpu.VMEM((2, D, TQ), _BF16),
            pltpu.VMEM((S, TQ), _F32),
            pltpu.VMEM((S, TQ), _F32),
            pltpu.VMEM((8, TQ), _F32),
            pltpu.VMEM((8, TQ), _F32),
            pltpu.VMEM((8, TQ), _F32),
            pltpu.VMEM((Dh, TQ), _F32),
            pltpu.VMEM((16, S), _F32),
            pltpu.VMEM((S, D), _F32),
            pltpu.VMEM((S, D), _BF16),
            pltpu.VMEM((D, F), _BF16),
            pltpu.VMEM((D, F), _BF16),
            pltpu.VMEM((F, D), _BF16),
            pltpu.SemaphoreType.DMA((S // TC + 7 + S // 128,)),
        ],
        compiler_params=pltpu.CompilerParams(
            vmem_limit_bytes=100 * 1024 * 1024,
        ),
    )(x2, A_wqkv, A_wo, B_w_r, B_w_gate, B_w_up, B_w_down)
    return out.reshape(B, S, D)
```

```python
import functools
import math

import jax
import jax.numpy as jnp
from jax import lax
import jax.experimental.pallas as pl
import jax.experimental.pallas.tpu as pltpu

_F32 = jnp.float32
_BF16 = jnp.bfloat16

_NT = (((1,), (1,)), ((), ()))


def _rb(v):
    return v.astype(_BF16).astype(_F32)


def _same(m, dep):
    return jnp.maximum(m, jnp.minimum(dep, m))


def _kernel(x_hbm, wqkv_hbm, wo_hbm, wr_ref, wg_hbm, wu_hbm, wd_hbm, o_hbm,
            x_scr, w3_v, wo_v, xn_scr, qt_scr, k_scr, vt_scr, wqvt_scr,
            wot_scr, at_scr, s0, s1, m0, m1, l_scr, oa_scr, r_scr, res_scr,
            o_scr, wg_v, wu_v, wd_v, sems,
            *, S, D, H, TQ, TC, KC, SKEW, DEP, DEPO, GU):
    Dh = D // H
    HG = 128 // Dh
    NG = D // 128
    NQ = S // TQ
    NC = S // KC
    NT = S // TC
    qscale = float(Dh) ** -0.5 * math.log2(math.e)
    sb, mb = (s0, s1), (m0, m1)

    def x_copy(c):
        rows = pl.ds(c * TC, TC)
        return pltpu.make_async_copy(x_hbm.at[rows, :], x_scr.at[rows, :],
                                     sems.at[c])

    def w3_copy(i):
        return pltpu.make_async_copy(wqkv_hbm.at[:, pl.ds(i * D, D)],
                                     w3_v.at[i], sems.at[NT + i])

    wo_copy = pltpu.make_async_copy(wo_hbm, wo_v, sems.at[NT + 3])
    ffn_copies = (pltpu.make_async_copy(wg_hbm, wg_v, sems.at[NT + 4]),
                  pltpu.make_async_copy(wu_hbm, wu_v, sems.at[NT + 5]),
                  pltpu.make_async_copy(wd_hbm, wd_v, sems.at[NT + 6]))

    def out_copy(i):
        rows = pl.ds(pl.multiple_of(i * 128, 128), 128)
        return pltpu.make_async_copy(o_scr.at[rows, :], o_hbm.at[rows, :],
                                     sems.at[NT + 7 + i])

    x_copy(0).start()
    w3_copy(1).start()
    x_copy(1).start()
    w3_copy(0).start()
    w3_copy(2).start()

    wr = jnp.broadcast_to(wr_ref[...].reshape(1, D), (16, D))

    def layernorm(c):
        rows = pl.ds(c * TC, TC)
        xf = x_scr[rows, :].astype(_F32)
        mu = jnp.mean(xf, axis=-1, keepdims=True)
        xc = xf - mu
        var = jnp.mean(xc * xc, axis=-1, keepdims=True)
        den = _rb(jnp.sqrt(_rb(_rb(var) + 1e-5)))
        xn = (_rb(xf - _rb(mu)) * (1.0 / den)).astype(_BF16)
        xn_scr[rows, :] = xn
        res_scr[rows, :] = xf + xn.astype(_F32)

    def router(c):
        rows = pl.ds(c * TC, TC)
        r_scr[:, rows] = _rb(lax.dot_general(wr, xn_scr[rows, :], _NT,
                                             preferred_element_type=_F32))

    def project_k(c, n=TC):
        rows = pl.ds(c * n, n)
        k = jnp.dot(xn_scr[rows, :], w3_v[1], preferred_element_type=_F32)
        k_scr[rows, :] = k.astype(_BF16)

    def project_q(c, n=TC):
        rows = pl.ds(c * n, n)
        qt = lax.dot_general(wqvt_scr[0:D, :], xn_scr[rows, :], _NT,
                             preferred_element_type=_F32)
        qt_scr[:, rows] = (qt * qscale).astype(_BF16)

    def project_v(c, n=TC):
        rows = pl.ds(c * n, n)
        vt = lax.dot_general(wqvt_scr[D:2 * D, :], xn_scr[rows, :], _NT,
                             preferred_element_type=_F32)
        vt_scr[:, rows] = vt.astype(_BF16)
        s1[rows, :] = jnp.zeros((n, TQ), _F32)

    x_copy(0).wait()
    for c in range(2, NT):
        x_copy(c).start()
    wo_copy.start()
    layernorm(0)
    w3_copy(1).wait()
    x_copy(1).wait()
    project_k(0)
    layernorm(1)
    project_k(1)
    w3_copy(0).wait()
    w3_copy(2).wait()
    wqvt_scr[0:D, :] = w3_v[0].astype(_F32).T.astype(_BF16)
    wqvt_scr[D:2 * D, :] = w3_v[2].astype(_F32).T.astype(_BF16)
    router(0)
    router(1)
    project_q(0)
    project_v(0)
    project_q(1)
    for c in range(2, NT):
        x_copy(c).wait()
    wo_copy.wait()
    for cp in ffn_copies:
        cp.start()
    wot_scr[...] = wo_v[...].astype(_F32).T.astype(_BF16)
    project_v(1)
    for c in range(2, NT):
        layernorm(c)
    for c in range(2, NT - 2):
        router(c)
        project_k(c)
        if c + 2 >= NT - 2:
            router(c + 2)
        project_q(c)
        project_v(c)
    for cp in ffn_copies:
        cp.wait()

    F = wg_v.shape[1]
    SUB = 128
    fill = []
    for c in range((NT - 2) * TC // SUB, NT * TC // SUB):
        fill += [functools.partial(f, c, SUB)
                 for f in (project_k, project_q, project_v)]

    def filler():
        if fill:
            fill.pop(0)()

    filler()
    r = r_scr[...]
    rmax = jnp.max(r, axis=-1, keepdims=True)
    col = lax.broadcasted_iota(jnp.int32, (16, S), 1)
    idx = jnp.min(jnp.where(r == rmax, col, S), axis=-1, keepdims=True)
    onehot = jnp.where(col == idx, 1.0, 0.0).astype(_BF16)
    xsel = None
    for i in range(2):
        cols = slice(i * S // 2, (i + 1) * S // 2)
        part = jnp.dot(onehot[:, cols], xn_scr[cols, :],
                       preferred_element_type=_F32)
        xsel = part if xsel is None else xsel + part
        filler()
    xsel = xsel.astype(_BF16)
    gus = []
    for i in range(2):
        cols = slice(i * F // 2, (i + 1) * F // 2)
        g = _rb(jnp.dot(xsel, wg_v[:, cols], preferred_element_type=_F32))
        g = _rb(g * _rb(jax.nn.sigmoid(g)))
        filler()
        u = _rb(jnp.dot(xsel, wu_v[:, cols], preferred_element_type=_F32))
        gus.append((g * u).astype(_BF16))
        filler()
    y = None
    for i in range(2):
        cols = slice(i * F // 2, (i + 1) * F // 2)
        part = jnp.dot(gus[i], wd_v[cols, :], preferred_element_type=_F32)
        y = part if y is None else y + part
        filler()
    y = _rb(_rb(y) * _rb(jax.nn.sigmoid(rmax)))
    idx_s = jnp.clip(jnp.min(idx), 0, S - 1)
    row = pl.ds(idx_s, 1)
    res_scr[row, :] = res_scr[row, :] + y[0:1, :]
    while fill:
        filler()
    s0[pl.ds(S - SKEW * KC, SKEW * KC), :] = jnp.zeros((SKEW * KC, TQ), _F32)
    m0[...] = jnp.zeros_like(m0)
    m1[...] = jnp.zeros_like(m1)
    l_scr[...] = jnp.ones_like(l_scr)
    oa_scr[...] = jnp.zeros_like(oa_scr)

    def run(qb, g, do_a, nslots, extra=()):
        extra = list(extra)
        h_base = g * HG
        gbase = qb * H + h_base
        lacc, oacc = l_scr[...], oa_scr[...]
        w = macc = mB = None
        hist, histo = [], []
        if do_a:
            q0 = pl.multiple_of(qb * TQ, TQ)
        for n in range(nslots):
            j, c = divmod(n, NC)
            if do_a:
                if c == 0:
                    jj = j % HG
                    c0 = pl.multiple_of((g + j // HG) * 128, 128)
                    r0a = pl.multiple_of((h_base + j) * Dh, Dh)
                    qrow = qt_scr[pl.ds(r0a, Dh), pl.ds(q0, TQ)]
                    parts = []
                    if jj > 0:
                        parts.append(jnp.zeros((jj * Dh, TQ), _BF16))
                    parts.append(qrow)
                    if jj < HG - 1:
                        parts.append(jnp.zeros(((HG - 1 - jj) * Dh, TQ), _BF16))
                    w = jnp.concatenate(parts, axis=0)
                    macc = None
                rows = pl.ds(c * KC, KC)
                s = jnp.dot(k_scr[rows, pl.ds(c0, 128)], w,
                            preferred_element_type=_F32)
                sb[j % 2][rows, :] = s
                for r in range(KC // 8):
                    sr = s[r * 8:(r + 1) * 8, :]
                    macc = sr if macc is None else jnp.maximum(macc, sr)
                if c == NC - 1:
                    mb[j % 2][...] = jnp.broadcast_to(
                        jnp.max(macc, axis=0, keepdims=True), (8, TQ))
            jb, cb = divmod(n - NC - SKEW, NC)
            gB = gbase + jb + 2 * H
            r0 = pl.multiple_of((gB % H) * Dh, Dh)
            if cb == 0 or mB is None:
                mB = mb[jb % 2][...]
            if cb == 0:
                lacc = None
                oacc = None
            mcur = mB
            if len(hist) >= DEP:
                mcur = _same(mcur, hist[-DEP])
            if len(histo) >= DEPO:
                mcur = _same(mcur, histo[-DEPO])
            rows = pl.ds(cb * KC, KC)
            p = jnp.exp2(sb[jb % 2][rows, :].reshape(KC // 8, 8, TQ)
                         - mcur[None]).reshape(KC, TQ)
            for r in reversed(range(KC // 8)):
                pr = p[r * 8:(r + 1) * 8, :]
                lacc = pr if lacc is None else lacc + pr
            hist.append(lacc)
            oc = jnp.dot(vt_scr[pl.ds(r0, Dh), rows], p.astype(_BF16),
                         preferred_element_type=_F32)
            oacc = oc if oacc is None else oacc + oc
            histo.append(oc[0:8, :])
            if cb == NC - 1:
                l = jnp.sum(lacc, axis=0, keepdims=True)
                par = (gB // H) % 2
                at_scr[par, pl.ds(r0, Dh), :] = (oacc / l).astype(_BF16)
            if extra and n % 4 == 3:
                extra.pop(0)()
        assert not extra
        l_scr[...] = lacc
        oa_scr[...] = oacc

    def finish_block(qb):
        par = qb % 2
        for t in range(TQ // 128):
            rows = pl.ds(pl.multiple_of(qb * TQ + t * 128, 128), 128)
            outt = jnp.dot(wot_scr[...], at_scr[par, :, t * 128:(t + 1) * 128],
                           preferred_element_type=_F32)
            o_scr[rows, :] = (res_scr[rows, :] + outt.T).astype(o_scr.dtype)
            out_copy(qb * (TQ // 128) + t).start()

    def finish_late(qb, k0):
        for t in range(TQ // 128):
            rows = pl.ds(qb * TQ + t * 128, 128)
            att = at_scr[qb % 2, k0:D, t * 128:(t + 1) * 128]
            out = jnp.dot(att.astype(_F32).T.astype(_BF16), wo_v[k0:D, :],
                          preferred_element_type=_F32)
            o_scr[rows, :] = (res_scr[rows, :] + out).astype(o_scr.dtype)
            out_copy(qb * (TQ // 128) + t).start()

    def early_proj(qb, k1, t):
        rows = pl.ds(qb * TQ + t * 128, 128)
        outt = jnp.dot(wot_scr[:, 0:k1],
                       at_scr[qb % 2, 0:k1, t * 128:(t + 1) * 128],
                       preferred_element_type=_F32)
        res_scr[rows, :] = res_scr[rows, :] + outt.T

    def body(t, carry):
        qb = t // (NG // GU)
        g = (t % (NG // GU)) * GU
        run(qb, g, True, GU * HG * NC)

        @pl.when(jnp.logical_and(g == 0, qb > 0))
        def _():
            finish_block(qb - 1)
        return carry

    lax.fori_loop(0, NQ * NG // GU, body, 0)
    k1 = D - 128
    run(NQ, 0, False, NC + SKEW,
        [functools.partial(early_proj, NQ - 1, k1, t) for t in range(TQ // 128)])
    finish_late(NQ - 1, k1)
    for i in range(S // 128):
        out_copy(i).wait()


@jax.jit
def pallas_parallel_sum__softmax_full_mha__moe_arch_mod__prompt_kernel(
    A_x: jax.Array,
    A_wqkv: jax.Array,
    A_wo: jax.Array,
    B_x: jax.Array,
    B_w_r: jax.Array,
    B_w_gate: jax.Array,
    B_w_up: jax.Array,
    B_w_down: jax.Array,
):
    del B_x
    B, S, D = A_x.shape
    assert B == 1
    F = B_w_gate.shape[1]
    H = 32
    TQ = 512
    TC = 256
    NQ = S // TQ
    Dh = D // H

    x2 = A_x.reshape(S, D)

    hbm = pl.BlockSpec(memory_space=pl.ANY)
    kern = functools.partial(_kernel, S=S, D=D, H=H, TQ=TQ, TC=TC, KC=128,
                             SKEW=4, DEP=2, DEPO=3, GU=1)
    out = pl.pallas_call(
        kern,
        in_specs=[hbm, hbm, hbm, pl.BlockSpec(memory_space=pltpu.VMEM),
                  hbm, hbm, hbm],
        out_specs=hbm,
        out_shape=jax.ShapeDtypeStruct((S, D), A_x.dtype),
        scratch_shapes=[
            pltpu.VMEM((S, D), _BF16),
            pltpu.VMEM((3, D, D), _BF16),
            pltpu.VMEM((D, D), _BF16),
            pltpu.VMEM((S, D), _BF16),
            pltpu.VMEM((D, S), _BF16),
            pltpu.VMEM((S, D), _BF16),
            pltpu.VMEM((D, S), _BF16),
            pltpu.VMEM((2 * D, D), _BF16),
            pltpu.VMEM((D, D), _BF16),
            pltpu.VMEM((2, D, TQ), _BF16),
            pltpu.VMEM((S, TQ), _F32),
            pltpu.VMEM((S, TQ), _F32),
            pltpu.VMEM((8, TQ), _F32),
            pltpu.VMEM((8, TQ), _F32),
            pltpu.VMEM((8, TQ), _F32),
            pltpu.VMEM((Dh, TQ), _F32),
            pltpu.VMEM((16, S), _F32),
            pltpu.VMEM((S, D), _F32),
            pltpu.VMEM((S, D), _BF16),
            pltpu.VMEM((D, F), _BF16),
            pltpu.VMEM((D, F), _BF16),
            pltpu.VMEM((F, D), _BF16),
            pltpu.SemaphoreType.DMA((S // TC + 7 + S // 128,)),
        ],
        compiler_params=pltpu.CompilerParams(
            vmem_limit_bytes=100 * 1024 * 1024,
        ),
    )(x2, A_wqkv, A_wo, B_w_r, B_w_gate, B_w_up, B_w_down)
    return out.reshape(B, S, D)
```
